```python
import jax
import jax.numpy as jnp

def _softmax(x, axis=-1):
    return jax.nn.softmax(x, axis=axis)
def _gelu(x):
    return jax.nn.gelu(x, approximate=True)
def _silu(x):
    return jax.nn.silu(x)
def _sigmoid(x):
    return jax.nn.sigmoid(x)
def _layernorm(x, axis=-1, eps=1e-5):
    m = jnp.mean(x, axis=axis, keepdims=True)
    v = jnp.var(x, axis=axis, keepdims=True)
    return (x - m) / jnp.sqrt(v + eps)
def _scatter_add(tgt, idx, src, axis=0):
    return tgt.at[idx].add(src)
def _segment_sum(src, seg, n):
    return jax.ops.segment_sum(src, seg, n)
class _Rng:
    def __init__(self, key):
        self._k = key
    def _next(self):
        self._k, sub = jax.random.split(self._k)
        return sub
    def normal(self, shape):
        return jax.random.normal(self._next(), shape, dtype=jnp.bfloat16)
    def randint(self, lo, hi, shape):
        return jax.random.randint(self._next(), shape, lo, hi, dtype=jnp.int32)
    def uniform(self, shape, lo=0.0, hi=1.0):
        return jax.random.uniform(self._next(), shape, jnp.bfloat16, lo, hi)
    def permutation(self, n):
        return jax.random.permutation(self._next(), n)


kernel_name = 'concat_heads__mha_block_cached__gqa_block_cached__near_ridge'

def _fwd_setup_inputs():
    _rng = _Rng(jax.random.key(int.from_bytes(__import__("os").urandom(4), "little")))
    _w = (lambda a: (lambda t: t.astype(jnp.bfloat16) if jnp.issubdtype(t.dtype, jnp.floating) else t)(jnp.asarray(a)))
    def _A_setup():
        B, Sq, D = 8, 224, 448
        H, Sk, Dh = 16, 512, 256
        return {
            "x": _w((lambda *s: _rng.normal(s) * 0.05)(B, Sq, D)),
            "k_cache": _w((lambda *s: _rng.normal(s) * 0.05)(B, H, Sk, Dh)),
            "v_cache": _w((lambda *s: _rng.normal(s) * 0.05)(B, H, Sk, Dh)),
            "wq": _w((lambda *s: _rng.normal(s) * 0.05)(D, H * Dh) * (D ** -0.5)),
            "wo": _w((lambda *s: _rng.normal(s) * 0.05)(H * Dh, D) * ((H * Dh) ** -0.5)),
        }
    _A_in = _A_setup()

    def _B_setup():
        B, Sq, D = 8, 224, 448
        Hq, Hkv, Sk, Dh = 16, 16, 512, 256
        assert Hq % Hkv == 0, (Hq, Hkv)
        return {
            "x": _w((lambda *s: _rng.normal(s) * 0.05)(B, Sq, D)),
            "k_cache": _w((lambda *s: _rng.normal(s) * 0.05)(B, Hkv, Sk, Dh)),
            "v_cache": _w((lambda *s: _rng.normal(s) * 0.05)(B, Hkv, Sk, Dh)),
            "wq": _w((lambda *s: _rng.normal(s) * 0.05)(D, Hq * Dh) * (D ** -0.5)),
            "wo": _w((lambda *s: _rng.normal(s) * 0.05)(Hq * Dh, D) * ((Hq * Dh) ** -0.5)),
        }
    _B_in = _B_setup()

    return {
        "A_x": _A_in["x"],
        "A_k_cache": _A_in["k_cache"],
        "A_v_cache": _A_in["v_cache"],
        "A_wq": _A_in["wq"],
        "A_wo": _A_in["wo"],
        "B_x": _B_in["x"],
        "B_k_cache": _B_in["k_cache"],
        "B_v_cache": _B_in["v_cache"],
        "B_wq": _B_in["wq"],
        "B_wo": _B_in["wo"],
    }

def _fwd_reference(A_x, A_k_cache, A_v_cache, A_wq, A_wo, B_x, B_k_cache, B_v_cache, B_wq, B_wo):
    def _A_ref(x, k_cache, v_cache, wq, wo):
        B, Sq, D = x.shape
        H, Dh = 16, 256
        q = (lambda x, *d: x.transpose(*d))((x @ wq).reshape(B, Sq, H, Dh), 0, 2, 1, 3)
        scores = jnp.einsum("bhqd,bhkd->bhqk", q, k_cache) * (Dh ** -0.5)
        p = _softmax(scores, axis=-1)
        o = jnp.einsum("bhqk,bhkd->bhqd", p, v_cache)
        return (lambda x, *d: x.transpose(*d))(o, 0, 2, 1, 3).reshape(B, Sq, H * Dh) @ wo

    def _B_ref(x, k_cache, v_cache, wq, wo):
        B, Sq, D = x.shape
        Hq, Dh = 16, 256
        Hkv = k_cache.shape[1]
        rep = Hq // Hkv
        q = (lambda x, *d: x.transpose(*d))((x @ wq).reshape(B, Sq, Hq, Dh), 0, 2, 1, 3)
        k = jnp.repeat(k_cache, rep, axis=1)
        v = jnp.repeat(v_cache, rep, axis=1)
        scores = jnp.einsum("bhqd,bhkd->bhqk", q, k) * (Dh ** -0.5)
        p = _softmax(scores, axis=-1)
        o = jnp.einsum("bhqk,bhkd->bhqd", p, v)
        return (lambda x, *d: x.transpose(*d))(o, 0, 2, 1, 3).reshape(B, Sq, Hq * Dh) @ wo

    a = _A_ref(A_x, A_k_cache, A_v_cache, A_wq, A_wo)
    b = _B_ref(B_x, B_k_cache, B_v_cache, B_wq, B_wo)
    return jnp.concatenate([a, b], axis=-1)


def setup_inputs():
    _inp = _fwd_setup_inputs()
    _gk = jax.random.fold_in(jax.random.key(int.from_bytes(__import__("os").urandom(4), "little")), 2**31 - 1)
    _shapes = [[8, 224, 896]]
    _dtypes = ['bfloat16']
    _gks = jax.random.split(_gk, len(_shapes))
    _gs = [jax.random.normal(k, s, dtype=jnp.dtype(d)) * 0.05 for k, s, d in zip(_gks, _shapes, _dtypes)]
    _inp["grad_out"] = _gs[0]
    return _inp

def reference(A_x, A_k_cache, A_v_cache, A_wq, A_wo, B_x, B_k_cache, B_v_cache, B_wq, B_wo, grad_out):
    _const = dict()
    def _f(*_d):
        return _fwd_reference(**{'A_x': _d[0], 'A_k_cache': _d[1], 'A_v_cache': _d[2], 'A_wq': _d[3], 'A_wo': _d[4], 'B_x': _d[5], 'B_k_cache': _d[6], 'B_v_cache': _d[7], 'B_wq': _d[8], 'B_wo': _d[9], **_const})
    _out, _vjp = jax.vjp(_f, A_x, A_k_cache, A_v_cache, A_wq, A_wo, B_x, B_k_cache, B_v_cache, B_wq, B_wo)
    _grads = _vjp(grad_out)
    _out0 = jnp.asarray(_out)
    return (_out0, *[jnp.asarray(_g) for _g in _grads])
```

```python
import jax
import jax.numpy as jnp
from jax import lax
import jax.experimental.pallas as pl
import jax.experimental.pallas.tpu as pltpu

B, SQ, D, H, SK, DH = 8, 224, 448, 16, 512, 256
HQ, HD, HK, HH = SQ // 2, D // 2, SK // 2, DH // 2
R = B * HQ
TILES = R // 128
UNITS = R // 16
GW = 512
STEPS = 2 * H
SCALE = DH ** -0.5
F32, BF16 = jnp.float32, jnp.bfloat16
NN = (((1,), (0,)), ((), ()))
NT = (((1,), (1,)), ((), ()))
TN = (((0,), (0,)), ((), ()))

QUADS = ((0, 0), (0, 1), (1, 0), (1, 1))
QUADS_T = ((0, 0), (1, 0), (0, 1), (1, 1))
B_TERMS = ((0, 3, 1), (0,), (1, 3, -1), (2, 0, -1), (3,), (0, 1, 1), (2, 3, 1))
ORDER = dict(q="1502436", s="1253046", o="1350246", do="3025146", dp="0153246", dq="5160324",
             dk="2450136", dv="2054361", dw="2540136")
PIPELINE = (("scores", 0), ("proj_q", 1), ("proj_do", 1), ("softmax", 0), ("out_head", -2),
            ("dx_head", -2), ("dprobs", 0), ("attn_o", 0), ("dsoftmax", 0), ("grad_v", 0),
            ("out_tail", -2), ("grad_q", 0), ("grad_k", 0), ("dx_tail", -2), ("send", 0))
OUT_SPLIT, DX_SPLIT = 6, 6
CACHE_GRAD_GROUPS = ((0, 7), (7, 8))
TAIL_GROUPS = ((0, 1), (1, 2), (2, 3), (3, 4), (4, 5), (5, 6), (6, 8))


def _dot(a, b, dims):
    return lax.dot_general(a, b, dims, preferred_element_type=F32)


def _a_comb(a11, a12, a21, a22):
    return [a11 + a22, a21 + a22, a11, a22, a11 + a12, a21 - a11, a12 - a22]


def _b_comb(b11, b12, b21, b22):
    return [b11 + b22, b11, b12 - b22, b21 - b11, b22, b11 + b12, b21 + b22]


def _c_comb(c11, c12, c21, c22):
    return [c11 + c22, c21 - c22, c12 + c22, c11 + c21, c12 - c11, c22, c11]


def _c_out(m):
    return (m[3] + m[0] - m[4] + m[6], m[2] + m[4], m[1] + m[3], m[5] - m[1] + m[0] + m[2])


def _a_out(n):
    return (n[0] - n[5] + n[2] + n[4], n[4] + n[6], n[1] + n[5], n[1] + n[3] + n[0] - n[6])


def _b_out(l):
    return (l[5] + l[0] + l[1] - l[3], l[2] + l[5], l[3] + l[6], l[4] - l[2] + l[0] + l[6])


def _bf16(xs):
    return [x.astype(BF16) for x in xs]


def _products(name, fn):
    m = {int(r): fn(int(r)) for r in ORDER[name]}
    return [m[r] for r in range(7)]


def _token_row(unit):
    return unit // (HQ // 16) * SQ + unit % (HQ // 16) * 16


def _kernel(xa, ka, va, wqa, woa, xb, kb, vb, wqb, wob, g,
            out, dxa, dka, dva, dwqa, dwoa, dxb, dkb, dvb, dwqb, dwob,
            x_s, g_s, kv_s, w_s, dkv_s, dw_s, out_s, dx_s, ax_s, cg_s, out_acc, dx_acc, ao, cdq, zero_s,
            sem_x, sem_w, sem_kv, sem_dkv, sem_dw, sem_fin):
    i = pl.program_id(0)
    slot = i % 2
    block = i // H
    first_head = i % H == 0

    def for_step(step, fn):
        for blk in range(2):
            @pl.when((step >= blk * H) & (step < (blk + 1) * H))
            def _():
                fn(blk, step - blk * H)

    def head_cols(head):
        return pl.ds(pl.multiple_of(head * DH, DH), DH)

    def wait_all(buf, sem):
        pltpu.make_async_copy(buf, buf, sem).wait()

    def token_copies(blk, b):
        rows = pl.ds(b * SQ, SQ) if blk == 0 else pl.ds(0, B * SQ)
        return [pltpu.make_async_copy((xa, xb)[blk].at[rows], x_s.at[blk, rows], sem_x.at[0, b]),
                pltpu.make_async_copy(g.at[rows, pl.ds(blk * (2 * D - GW), GW)], g_s.at[blk, rows],
                                      sem_x.at[1, b])]

    def result_copies(blk, b0=0, b1=B):
        rows = pl.ds(b0 * SQ, (b1 - b0) * SQ)
        cols = pl.ds(0, 2 * D - GW) if blk == 0 else pl.ds(2 * D - GW, GW)
        return [pltpu.make_async_copy(dx_s.at[rows], (dxa, dxb)[blk].at[rows], sem_fin.at[0, b0]),
                pltpu.make_async_copy(out_s.at[rows, cols], out.at[rows, cols], sem_fin.at[1, b0])]

    def start_inputs(step):
        def start(blk, head):
            for n, w in enumerate(((wqa, woa), (wqb, wob))[blk]):
                pltpu.make_async_copy(w.at[:, head_cols(head)], w_s.at[step % 2, n], sem_w.at[step % 2]).start()
            for n, t in enumerate(((ka, va), (kb, vb))[blk]):
                pltpu.make_async_copy(t.at[:, head], kv_s.at[step % 2, n],
                                      sem_kv.at[step % 2]).start(priority=n)
        for_step(step, start)

    def start_cache_grads(b0, b1):
        def start(blk, head):
            for n, t in enumerate(((dka, dva), (dkb, dvb))[blk]):
                pltpu.make_async_copy(dkv_s.at[slot, n, b0:b1], t.at[b0:b1, head], sem_dkv.at[slot]).start()
        for_step(i, start)

    def start_weight_grads():
        def start(blk, head):
            for n, t in enumerate(((dwqa, dwoa), (dwqb, dwob))[blk]):
                pltpu.make_async_copy(dw_s.at[slot, n], t.at[:, head_cols(head)], sem_dw.at[slot]).start()
        for_step(i, start)

    def wait_inputs(sl):
        wait_all(w_s.at[sl], sem_w.at[sl])
        wait_all(kv_s.at[sl], sem_kv.at[sl])

    def wait_outputs(sl):
        wait_all(dkv_s.at[sl], sem_dkv.at[sl])
        wait_all(dw_s.at[sl], sem_dw.at[sl])

    def convert(src_blk, dst_blk, src_row, dst_row, n, g_off):
        lane = lax.broadcasted_iota(jnp.int32, (n // 2, 128), 1)

        def window(t, off):
            t, off = t[off // 128:], off % 128
            if off == 0:
                return t[0], t[1]
            t = [pltpu.roll(v, 128 - off, 1) for v in t[:3]]
            keep = lane < 128 - off
            return jnp.where(keep, t[0], t[1]), jnp.where(keep, t[1], t[-1])

        for src, off, comb, dst, plain in ((x_s, 0, _a_comb, ax_s, (2, 3)), (g_s, g_off, _c_comb, cg_s, (6, 5))):
            quads = []
            for a in range(2):
                rows = pl.ds(pl.multiple_of(src_row + a * HQ, 16), n)
                t = [src[src_blk, rows, c:min(c + 128, src.shape[-1])] for c in range(0, GW, 128)]
                if src is x_s:
                    t[3] = jnp.concatenate([t[3], jnp.zeros((n, GW - D), BF16)], axis=1)
                t = [pltpu.bitcast(v, jnp.uint32) for v in t]
                quads += [window(t, off), window(t, off + HD)]
            for c in range(2):
                part = [pltpu.bitcast(t[c], BF16) for t in quads]
                copies = dict(zip(plain, (part[0], part[3])))
                for r, t in enumerate(comb(*[t.astype(F32) for t in part])):
                    dst[dst_blk, r, c, pl.ds(pl.multiple_of(dst_row, 16), n)] = (
                        copies[r] if r in copies else t.astype(BF16))

    def finish(blk, j, a, out_col, active=None):
        for acc, recomb, dst, col in ((dx_acc, _a_out, dx_s, 0), (out_acc, _c_out, out_s, out_col)):
            quads = recomb([acc[blk, j, r] for r in range(7)])
            if isinstance(a, int):
                parts = list(quads[2 * a:2 * a + 2])
            else:
                parts = [jnp.where(a == 0, u, v) for u, v in zip(quads[:2], quads[2:])]
            if col % 128:
                parts = [jnp.zeros((col % 128, 128), F32)] + parts
            t = jnp.concatenate(parts, axis=0).T
            for u in range(8):
                row = _token_row(j * 8 + u) + a * HQ
                if active is not None:
                    row = pl.multiple_of(jnp.where(active, row, B * SQ + u * 16), 16)
                dst[pl.ds(row, 16), col:col + D] = t[u * 16:(u + 1) * 16, col % 128:].astype(BF16)

    @pl.when(i == 0)
    def _():
        for n in range(14):
            zero_s[n] = 0
        for b in range(B):
            for c in token_copies(0, b):
                c.start()
        start_inputs(i)

        def body(b, carry):
            for c in token_copies(0, b):
                c.wait()
            convert(0, 0, b * SQ, b * HQ, HQ, 0)
            return carry
        lax.fori_loop(0, B, body, 0)
        wait_inputs(0)
        start_inputs(i + 1)
        for c in token_copies(1, 0):
            c.start()

    @pl.when(i == 2)
    def _():
        for c in token_copies(1, 0):
            c.wait()

    @pl.when(i >= 1)
    def _():
        wait_inputs(slot)

    @pl.when(i >= 2)
    def _():
        wait_outputs(slot)

    wq = w_s[slot, 0].astype(F32) * SCALE
    bwq = _bf16(_b_comb(*[wq[a * HD:(a + 1) * HD, c * HH:(c + 1) * HH] for a, c in QUADS]))
    wo = w_s[slot, 1].astype(F32)
    bwo = _bf16(_b_comb(*[wo[a * HD:(a + 1) * HD, c * HH:(c + 1) * HH] for a, c in QUADS_T]))
    slots = [slot + zero_s[n] for n in range(14)]
    st = [dict() for _ in range(B)]

    def rows_of(b):
        return slice(b * HQ, (b + 1) * HQ)

    def cache_comb(n, b, quads, use, r):
        def load(q):
            a, c = quads[q]
            return kv_s[slots[7 * use + r], n, b, a * HK:(a + 1) * HK, c * HH:(c + 1) * HH]
        t = B_TERMS[r]
        if len(t) == 1:
            return load(t[0])
        x, y = load(t[0]).astype(F32), load(t[1]).astype(F32)
        return (x + y if t[2] > 0 else x - y).astype(BF16)

    def token_comb(ref, r, rows):
        return jnp.concatenate([ref[block, r, 0, rows], ref[block, r, 1, rows, :HD - 128]], axis=1)

    def proj_q(b):
        q = _c_out(_products("q", lambda r: _dot(token_comb(ax_s, r, rows_of(b)), bwq[r], NN)))
        st[b]["aq"] = _bf16(_a_comb(*q))

    def proj_do(b):
        do = _a_out(_products("do", lambda r: _dot(token_comb(cg_s, r, rows_of(b)), bwo[r], NN)))
        st[b]["cdo"] = _bf16(_c_comb(*do))

    def scores(b):
        st[b]["s"] = _c_out(_products(
            "s", lambda r: _dot(st[b]["aq"][r], cache_comb(0, b, QUADS_T, 0, r), NT)))

    def dprobs(b):
        st[b]["dp"] = _a_out(_products(
            "dp", lambda r: _dot(st[b]["cdo"][r], cache_comb(1, b, QUADS, 0, r), NT)))

    def softmax(b):
        s, p = st[b]["s"], []
        for s0, s1 in (s[:2], s[2:]):
            m = jnp.max(jnp.maximum(s0, s1), axis=1, keepdims=True)
            l = jnp.sum(jnp.exp(s0 - m) + jnp.exp(s1 - m), axis=1, keepdims=True)
            lse = m + jnp.log(l)
            p += [jnp.exp(s0 - lse), jnp.exp(s1 - lse)]
        st[b]["p"], st[b]["ap"] = p, _bf16(_a_comb(*p))

    def dsoftmax(b):
        p, dp, ds = st[b]["p"], st[b]["dp"], []
        for a in (0, 2):
            delta = jnp.sum(p[a] * dp[a] + p[a + 1] * dp[a + 1], axis=1, keepdims=True)
            ds += [p[a] * (dp[a] - delta), p[a + 1] * (dp[a + 1] - delta)]
        st[b]["cds"] = _bf16(_c_comb(*ds))

    def attn_o(b):
        o = _c_out(_products("o", lambda r: _dot(st[b]["ap"][r], cache_comb(1, b, QUADS, 1, r), NN)))
        for r, t in enumerate(_bf16(_a_comb(*o))):
            ao[r, rows_of(b)] = t

    def grad_q(b):
        dq = _a_out(_products("dq", lambda r: _dot(st[b]["cds"][r], cache_comb(0, b, QUADS_T, 1, r), NN)))
        for r, t in enumerate(_bf16(_c_comb(*dq))):
            cdq[r, rows_of(b)] = t

    def cache_grad(n, b, lhs, rhs, quads):
        grad = dict(zip(quads, _b_out(_products(("dk", "dv")[n], lambda r: _dot(lhs[r], rhs[r], TN)))))
        for a in range(2):
            dkv_s[slot, n, b, a * HK:(a + 1) * HK] = jnp.concatenate(
                [grad[a, 0], grad[a, 1]], axis=1).astype(BF16)

    def send(b):
        for b0, b1 in CACHE_GRAD_GROUPS:
            if b1 == b + 1:
                start_cache_grads(b0, b1)

    def accumulate(acc, w, act, j, rs):
        for r in rs:
            acc[block, j, r] = (jnp.where(first_head, 0.0, acc[block, j, r])
                                + _dot(w[r], act[r, j * 128:(j + 1) * 128], NT))

    def weight_grad(n, lhs, rhs, quads, scale):
        grad = _b_out(_products("dw", lambda r: _dot(token_comb(lhs, r, slice(None)), rhs[r], TN)))
        grad = dict(zip(quads, grad))
        for a in range(2):
            t = jnp.concatenate([grad[a, 0], grad[a, 1]], axis=1)
            dw_s[slot, n, a * HD:(a + 1) * HD] = (t * scale if scale else t).astype(BF16)

    batch_tasks = dict(
        proj_q=proj_q, proj_do=proj_do, scores=scores, dprobs=dprobs, softmax=softmax,
        dsoftmax=dsoftmax, attn_o=attn_o, grad_q=grad_q, send=send,
        grad_k=lambda b: cache_grad(0, b, st[b]["cds"], st[b]["aq"], QUADS_T),
        grad_v=lambda b: cache_grad(1, b, st[b]["ap"], st[b]["cdo"], QUADS))
    tile_tasks = dict(
        out_head=lambda j: accumulate(out_acc, bwo, ao, j, range(OUT_SPLIT)),
        out_tail=lambda j: accumulate(out_acc, bwo, ao, j, range(OUT_SPLIT, 7)),
        dx_head=lambda j: accumulate(dx_acc, bwq, cdq, j, range(DX_SPLIT)),
        dx_tail=lambda j: accumulate(dx_acc, bwq, cdq, j, range(DX_SPLIT, 7)))
    for t in range(-2, B + 2):
        for name, offset in PIPELINE:
            if name in batch_tasks and 0 <= t + offset < B:
                batch_tasks[name](t + offset)
            if name in tile_tasks and 0 <= t + offset < TILES:
                tile_tasks[name](t + offset)
    weight_grad(1, cg_s, ao, QUADS_T, None)
    weight_grad(0, ax_s, cdq, QUADS, SCALE)

    part = jnp.clip(i - 2, 0, UNITS // 4 - 1)
    for u in range(4):
        unit = part * 4 + u
        convert(jnp.where(i >= 2, 1, 0), 1 - block, _token_row(unit), unit * 16, 16, GW - D)
    part = jnp.clip(i - H, 0, 2 * TILES - 1)
    finish(0, part // 2, part % 2, 0, (i >= H) & (i < H + 2 * TILES))

    start_inputs(i + 2)
    start_weight_grads()

    @pl.when(i == H + 2 * TILES)
    def _():
        for c in result_copies(0):
            c.start()

    @pl.when(i == STEPS - 1)
    def _():
        for c in result_copies(0):
            c.wait()
        for j in range(TILES):
            for a in range(2):
                finish(1, j, a, D)
            for b0, b1 in TAIL_GROUPS:
                if (j + 1) * 128 >= b1 * HQ > j * 128:
                    for c in result_copies(1, b0, b1):
                        c.start()
        wait_outputs(0)
        wait_outputs(1)
        for b0, b1 in TAIL_GROUPS:
            for c in result_copies(1, b0, b1):
                c.wait()


@jax.jit
def pallas_concat_heads__mha_block_cached__gqa_block_cached__near_ridge_kernel(
    A_x: jax.Array,
    A_k_cache: jax.Array,
    A_v_cache: jax.Array,
    A_wq: jax.Array,
    A_wo: jax.Array,
    B_x: jax.Array,
    B_k_cache: jax.Array,
    B_v_cache: jax.Array,
    B_wq: jax.Array,
    B_wo: jax.Array,
    grad_out: jax.Array,
):
    sds = jax.ShapeDtypeStruct
    block_out = [sds((B * SQ, D), BF16), sds((B, H, SK, DH), BF16), sds((B, H, SK, DH), BF16),
                 sds((D, H * DH), BF16), sds((D, H * DH), BF16)]
    hbm = pl.BlockSpec(memory_space=pl.ANY)
    vmem, dma = pltpu.VMEM, pltpu.SemaphoreType.DMA
    res = pl.pallas_call(
        _kernel,
        grid=(STEPS,),
        in_specs=[hbm] * 11,
        out_specs=[hbm] * 11,
        out_shape=[sds((B * SQ, 2 * D), BF16)] + block_out + block_out,
        scratch_shapes=[
            vmem((2, B * SQ, D), BF16), vmem((2, B * SQ, GW), BF16),
            vmem((2, 2, B, SK, DH), BF16), vmem((2, 2, D, DH), BF16),
            vmem((2, 2, B, SK, DH), BF16), vmem((2, 2, D, DH), BF16),
            vmem((B * SQ + 128, 2 * D), BF16), vmem((B * SQ + 128, D), BF16),
            vmem((2, 7, 2, R, 128), BF16), vmem((2, 7, 2, R, 128), BF16),
            vmem((2, TILES, 7, HD, 128), F32), vmem((2, TILES, 7, HD, 128), F32),
            vmem((7, R, HH), BF16), vmem((7, R, HH), BF16),
            pltpu.SMEM((14,), jnp.int32),
            dma((2, B)), dma((2,)), dma((2,)), dma((2,)), dma((2,)), dma((2, B)),
        ],
        compiler_params=pltpu.CompilerParams(
            dimension_semantics=("arbitrary",),
            vmem_limit_bytes=120 * 1024 * 1024,
            disable_bounds_checks=True),
    )(A_x.reshape(B * SQ, D), A_k_cache, A_v_cache, A_wq, A_wo.T,
      B_x.reshape(B * SQ, D), B_k_cache, B_v_cache, B_wq, B_wo.T,
      grad_out.reshape(B * SQ, 2 * D))
    out, dxa, dka, dva, dwqa, dwoa, dxb, dkb, dvb, dwqb, dwob = res
    return (out.reshape(B, SQ, 2 * D), dxa.reshape(B, SQ, D), dka, dva, dwqa, dwoa.T,
            dxb.reshape(B, SQ, D), dkb, dvb, dwqb, dwob.T)
```
